```python
import jax
import jax.numpy as jnp

def _softmax(x, axis=-1):
    return jax.nn.softmax(x, axis=axis)

def _gelu(x):
    return jax.nn.gelu(x, approximate=True)

def _silu(x):
    return jax.nn.silu(x)

def _sigmoid(x):
    return jax.nn.sigmoid(x)

def _layernorm(x, axis=-1, eps=1e-05):
    m = jnp.mean(x, axis=axis, keepdims=True)
    v = jnp.var(x, axis=axis, keepdims=True)
    return (x - m) / jnp.sqrt(v + eps)

def _scatter_add(tgt, idx, src, axis=0):
    return tgt.at[idx].add(src)

def _segment_sum(src, seg, n):
    return jax.ops.segment_sum(src, seg, n)

class _Rng:

    def __init__(self, key):
        self._k = key

    def _next(self):
        self._k, sub = jax.random.split(self._k)
        return sub

    def normal(self, shape):
        return jax.random.normal(self._next(), shape, dtype=jnp.bfloat16)

    def randint(self, lo, hi, shape):
        return jax.random.randint(self._next(), shape, lo, hi, dtype=jnp.int32)

    def uniform(self, shape, lo=0.0, hi=1.0):
        return jax.random.uniform(self._next(), shape, jnp.bfloat16, lo, hi)

    def permutation(self, n):
        return jax.random.permutation(self._next(), n)
kernel_name = 'interleave_layers__linear_kernel_hedgehog__memory_aug_recurrent_mem_tr__prompt'

def setup_inputs():
    _rng = _Rng(jax.random.key(int.from_bytes(__import__("os").urandom(4), "little")))
    _w = lambda a: (lambda t: t.astype(jnp.bfloat16) if jnp.issubdtype(t.dtype, jnp.floating) else t)(jnp.asarray(a))

    def _A_setup():
        B, S, D, H = (1, 2048, 640, 32)
        Dh = D // H
        return {'x': _w((lambda *s: _rng.normal(s) * 0.05)(B, S, D)), 'wqkv': _w((lambda *s: _rng.normal(s) * 0.05)(D, 3 * D)), 'w_phi': _w((lambda *s: _rng.normal(s) * 0.05)(H, Dh, Dh) * Dh ** (-0.5)), 'wo': _w((lambda *s: _rng.normal(s) * 0.05)(D, D))}
    _A_in = _A_setup()

    def _B_setup():
        B, S, Dm = (1, 2048, 640)
        H, Dh = (32, 192)
        M, seg = (8, 32)
        seg = min(seg, S)
        S = S // seg * seg
        return {'x': _w((lambda *s: _rng.normal(s) * 0.05)(B, S, Dm)), 'mem0': _w((lambda *s: _rng.normal(s) * 0.05)(B, M, Dm)), 'Wq': _w((lambda *s: _rng.normal(s) * 0.05)(Dm, H, Dh) * Dm ** (-0.5)), 'Wk': _w((lambda *s: _rng.normal(s) * 0.05)(Dm, H, Dh) * Dm ** (-0.5)), 'Wv': _w((lambda *s: _rng.normal(s) * 0.05)(Dm, H, Dh) * Dm ** (-0.5)), 'Wo': _w((lambda *s: _rng.normal(s) * 0.05)(H, Dh, Dm) * (H * Dh) ** (-0.5)), 'seg_len': seg}
    _B_in = _B_setup()
    return {'A_x': _A_in['x'], 'A_wqkv': _A_in['wqkv'], 'A_w_phi': _A_in['w_phi'], 'A_wo': _A_in['wo'], 'B_x': _B_in['x'], 'B_mem0': _B_in['mem0'], 'B_Wq': _B_in['Wq'], 'B_Wk': _B_in['Wk'], 'B_Wv': _B_in['Wv'], 'B_Wo': _B_in['Wo'], 'B_seg_len': _B_in['seg_len']}

def reference(A_x, A_wqkv, A_w_phi, A_wo, B_x, B_mem0, B_Wq, B_Wk, B_Wv, B_Wo, B_seg_len):

    def _A_ref(x, wqkv, w_phi, wo):
        B, S, D = x.shape
        H = 32
        Dh = D // H
        qkv = (lambda x, *d: x.transpose(*d))((x @ wqkv).reshape(B, S, 3, H, Dh), 2, 0, 3, 1, 4)
        q, k, v = (qkv[0], qkv[1], qkv[2])
        pq = jnp.einsum('bhsd,hdf->bhsf', q, w_phi)
        pk = jnp.einsum('bhsd,hdf->bhsf', k, w_phi)
        phi_q = jnp.concatenate([_softmax(pq, axis=-1), _softmax(-pq, axis=-1)], axis=-1)
        phi_k = jnp.concatenate([_softmax(pk, axis=-1), _softmax(-pk, axis=-1)], axis=-1)
        kv = jnp.einsum('bhsf,bhsd->bhfd', phi_k, v)
        z = jnp.einsum('bhsf->bhf', phi_k)
        num = jnp.einsum('bhqf,bhfd->bhqd', phi_q, kv)
        den = jnp.einsum('bhqf,bhf->bhq', phi_q, z)[..., None] + 1e-06
        o = num / den
        return (lambda x, *d: x.transpose(*d))(o, 0, 2, 1, 3).reshape(B, S, D) @ wo

    def _B_ref(x, mem0, Wq, Wk, Wv, Wo, seg_len):
        B, S, Dm = x.shape
        H, Dh = (Wq.shape[1], Wq.shape[2])
        M = mem0.shape[1]
        scale = Dh ** (-0.5)
        n_seg = S // seg_len
        L = M + seg_len
        idx = jnp.arange(L)
        mask = (idx[:, None] < M) | (idx[:, None] >= idx[None, :])
        mem = mem0
        outs = []
        for s in range(n_seg):
            xs = x[:, s * seg_len:(s + 1) * seg_len, :].copy()
            h = jnp.concatenate([mem, xs], axis=1)
            q = jnp.einsum('btd,dhe->bhte', h, Wq)
            k = jnp.einsum('btd,dhe->bhte', h, Wk)
            v = jnp.einsum('btd,dhe->bhte', h, Wv)
            scores = jnp.einsum('bhqe,bhke->bhqk', q, k) * scale
            scores = jnp.where(mask[None, None], scores, -1000000000.0)
            p = _softmax(scores, axis=-1)
            o = jnp.einsum('bhqk,bhke->bhqe', p, v)
            o = jnp.einsum('bhte,hed->btd', o, Wo)
            mem = o[:, :M, :].copy()
            outs.append(o[:, M:, :])
        return jnp.concatenate(outs, axis=1)
    x = A_x
    x = x + _A_ref(_layernorm(x, axis=-1), A_wqkv, A_w_phi, A_wo)
    x = x + _B_ref(_layernorm(x, axis=-1), B_mem0, B_Wq, B_Wk, B_Wv, B_Wo, B_seg_len)
    x = x + _A_ref(_layernorm(x, axis=-1), A_wqkv, A_w_phi, A_wo)
    x = x + _B_ref(_layernorm(x, axis=-1), B_mem0, B_Wq, B_Wk, B_Wv, B_Wo, B_seg_len)
    return x
```

```python
import functools

import jax
import jax.numpy as jnp
import jax.experimental.pallas as pl
import jax.experimental.pallas.tpu as pltpu

F32 = jnp.float32
BF16 = jnp.bfloat16

S, D = 2048, 640
HA, FA = 32, 20
HB, EB = 32, 192
M, SEG = 8, 32
L = M + SEG
TA = 256
PW = 2 * EB
NP = HB // 2

NT = (((1,), (1,)), ((), ()))
NN = (((1,), (0,)), ((), ()))
TN = (((0,), (0,)), ((), ()))


def _dot(a, b, dims=NN):
    return jax.lax.dot_general(a, b, dims, preferred_element_type=F32)


def _iota(shape, axis):
    return jax.lax.broadcasted_iota(jnp.int32, shape, axis)


def _rb(x):
    return x.astype(BF16).astype(F32)


def _ln(x):
    m = jnp.mean(x, axis=-1, keepdims=True)
    c = x - m
    v = jnp.mean(c * c, axis=-1, keepdims=True)
    return c * jax.lax.rsqrt(v + 1e-05)


def _fold(cols, op):
    r = cols[0]
    for c in cols[1:]:
        r = op(r, c)
    r = op(r, pltpu.roll(r, 64, 1))
    return op(r, pltpu.roll(r, 32, 1))


def _phi(p):
    cols = [p[:, j * 128:(j + 1) * 128] for j in range(5)]
    mx = _fold(cols, jnp.maximum)
    mn = _fold(cols, jnp.minimum)
    ep = [jnp.exp(c - mx) for c in cols]
    en = [jnp.exp(mn - c) for c in cols]
    rp = 1.0 / _fold(ep, jnp.add)
    rn = 1.0 / _fold(en, jnp.add)
    return [e * rp for e in ep] + [e * rn for e in en]


def _kernel(x_ref, wqkv_ref, wphi_ref, woa_ref, mem0_ref, wq_hbm, wk_hbm, wv_hbm, wo_hbm,
            o_ref, xs, xn, wa, wop, kvt, wq, wk, wv, wo, sems):
    copies = [pltpu.make_async_copy(s, d, sems.at[i]) for i, (s, d) in enumerate(
        ((wq_hbm, wq), (wk_hbm, wk), (wv_hbm, wv), (wo_hbm, wo)))]
    for c in copies:
        c.start()

    r = _iota((D, D), 0)
    c = _iota((D, D), 1)
    same = (r // FA) == (c % HA)
    sel = ((_iota((D, 32), 0) % FA) == _iota((D, 32), 1)).astype(BF16)
    rr = jnp.concatenate([wphi_ref[...], jnp.zeros((32 - FA, D), BF16)], axis=0)
    bmat = jnp.where(same, _dot(sel, rr), 0.0).astype(BF16)
    perm = jnp.logical_and(same, (r % FA) == (c // HA)).astype(BF16)
    wa[:, 0:D] = _dot(wqkv_ref[:, 0:D], bmat).astype(BF16)
    wa[:, D:2 * D] = _dot(wqkv_ref[:, D:2 * D], bmat).astype(BF16)
    wa[:, 2 * D:3 * D] = _dot(wqkv_ref[:, 2 * D:3 * D], perm).astype(BF16)
    wop[...] = _dot(perm, woa_ref[...], TN).astype(BF16)
    xs[...] = x_ref[...].astype(F32)

    def layer_a():
        kvt[...] = jnp.zeros_like(kvt)

        def keys(t, z):
            rows = pl.ds(pl.multiple_of(t * TA, TA), TA)
            h = _ln(xs[rows, :]).astype(BF16)
            xn[rows, :] = h.astype(F32)
            pkv = _dot(h, wa[:, D:3 * D])
            phi = jnp.concatenate(_phi(pkv[:, 0:D]), axis=1)
            kvt[...] += _dot(pkv[:, D:2 * D].astype(BF16), phi.astype(BF16), TN)
            return z + jnp.sum(phi, axis=0, keepdims=True)

        z = jax.lax.fori_loop(0, S // TA, keys, jnp.zeros((1, 2 * D), F32))
        msk = (_iota((D, 2 * D), 0) % HA) == (_iota((D, 2 * D), 1) % HA)
        kvb = jnp.where(msk, kvt[...], 0.0).astype(BF16)
        kw = _dot(kvb, wop[...], TN).astype(BF16)

        def queries(t, carry):
            rows = pl.ds(pl.multiple_of(t * TA, TA), TA)
            pq = _dot(xn[rows, :].astype(BF16), wa[:, 0:D])
            ph = _phi(pq)
            den = _fold([p * z[:, j * 128:(j + 1) * 128] for j, p in enumerate(ph)],
                        jnp.add) + 1e-06
            rd = 1.0 / den
            phn = jnp.concatenate([p * rd for p in ph], axis=1).astype(BF16)
            x = xs[rows, :] + _dot(phn, kw)
            xs[rows, :] = x
            xn[rows, :] = _rb(_ln(x))
            return carry

        jax.lax.fori_loop(0, S // TA, queries, 0)

    def layer_b():
        row = _iota((L, 2 * L), 0)
        col = _iota((L, 2 * L), 1)
        first = col < L
        keyi = jnp.where(first, col, col - L)
        vis = jnp.logical_or(row < M, row >= keyi)
        lane_a = _iota((L, PW), 1) < EB
        scale = EB ** (-0.5)

        def proj(h, p):
            sl = slice(p * PW, (p + 1) * PW)
            return _dot(h, wq[sl, :], NT), _dot(h, wk[sl, :], NT), _dot(h, wv[sl, :], NT)

        def bd(a):
            return jnp.concatenate([jnp.where(lane_a, a, 0.0), jnp.where(lane_a, 0.0, a)],
                                   axis=0).astype(BF16)

        def scores(q, k):
            s = _dot(_rb(q), bd(k), NT) * scale
            s = jnp.where(vis, s, -1000000000.0)
            ma = jnp.max(jnp.where(first, s, -jnp.inf), axis=-1, keepdims=True)
            mb = jnp.max(jnp.where(first, -jnp.inf, s), axis=-1, keepdims=True)
            e = jnp.exp(s - jnp.where(first, ma, mb))
            la = jnp.sum(jnp.where(first, e, 0.0), axis=-1, keepdims=True)
            lb = jnp.sum(jnp.where(first, 0.0, e), axis=-1, keepdims=True)
            return _rb(e / jnp.where(first, la, lb))

        def step(s, mem):
            rows = pl.ds(pl.multiple_of(s * SEG, SEG), SEG)
            h = jnp.concatenate([mem, xn[rows, :]], axis=0)
            qkv, pp, oo = {}, {}, {}
            acc = None
            LAG = 3
            for i in range(NP + 2 + LAG):
                if i < NP:
                    qkv[i] = proj(h, i)
                if 0 <= i - 1 < NP:
                    pp[i - 1] = scores(qkv[i - 1][0], qkv[i - 1][1])
                if 0 <= i - 2 < NP:
                    oo[i - 2] = _rb(_dot(pp.pop(i - 2), bd(qkv.pop(i - 2)[2])))
                j = i - 2 - LAG
                if 0 <= j < NP:
                    d = _dot(oo.pop(j), wo[j * PW:(j + 1) * PW, :])
                    acc = d if acc is None else acc + d
            xs[rows, :] = xs[rows, :] + acc[M:, :]
            return _rb(acc[:M, :])

        jax.lax.fori_loop(0, S // SEG, step, mem0_ref[...].astype(F32))

    def block(it, carry):
        layer_a()

        @pl.when(it == 0)
        def _():
            for cp in copies:
                cp.wait()

        layer_b()
        return carry

    jax.lax.fori_loop(0, 2, block, 0)
    o_ref[...] = xs[...].astype(o_ref.dtype)


@functools.partial(jax.jit, static_argnames=("B_seg_len",))
def pallas_interleave_layers__linear_kernel_hedgehog__memory_aug_recurrent_mem_tr__prompt_kernel(
    A_x, A_wqkv, A_w_phi, A_wo, B_x, B_mem0, B_Wq, B_Wk, B_Wv, B_Wo, B_seg_len,
):
    del B_x
    assert B_seg_len == SEG
    tr = lambda w: jnp.transpose(w, (1, 2, 0)).reshape(HB * EB, D)
    vm = pl.BlockSpec(memory_space=pltpu.VMEM)
    hbm = pl.BlockSpec(memory_space=pl.ANY)
    wshape = pltpu.VMEM((HB * EB, D), BF16)
    out = pl.pallas_call(
        _kernel,
        out_shape=jax.ShapeDtypeStruct((S, D), A_x.dtype),
        in_specs=[vm] * 5 + [hbm] * 4,
        out_specs=vm,
        scratch_shapes=[
            pltpu.VMEM((S, D), F32), pltpu.VMEM((S, D), F32),
            pltpu.VMEM((D, 3 * D), BF16), pltpu.VMEM((D, D), BF16),
            pltpu.VMEM((D, 2 * D), F32),
            wshape, wshape, wshape, wshape,
            pltpu.SemaphoreType.DMA((4,)),
        ],
        compiler_params=pltpu.CompilerParams(vmem_limit_bytes=100 * 1024 * 1024),
    )(
        A_x.reshape(S, D), A_wqkv,
        jnp.transpose(A_w_phi, (1, 2, 0)).reshape(FA, FA * HA), A_wo,
        B_mem0.reshape(M, D), tr(B_Wq), tr(B_Wk), tr(B_Wv), B_Wo.reshape(HB * EB, D),
    )
    return out.reshape(A_x.shape)
```

```python
import functools

import jax
import jax.numpy as jnp
import jax.experimental.pallas as pl
import jax.experimental.pallas.tpu as pltpu

F32 = jnp.float32
BF16 = jnp.bfloat16

S, D = 2048, 640
HA, FA = 32, 20
HB, EB = 32, 192
M, SEG = 8, 32
L = M + SEG
TA = 256
PW = 2 * EB
NP = HB // 2

NT = (((1,), (1,)), ((), ()))
NN = (((1,), (0,)), ((), ()))
TN = (((0,), (0,)), ((), ()))


def _dot(a, b, dims=NN):
    return jax.lax.dot_general(a, b, dims, preferred_element_type=F32)


def _iota(shape, axis):
    return jax.lax.broadcasted_iota(jnp.int32, shape, axis)


def _rb(x):
    return x.astype(BF16).astype(F32)


def _ln(x):
    m = jnp.mean(x, axis=-1, keepdims=True)
    c = x - m
    v = jnp.mean(c * c, axis=-1, keepdims=True)
    return c * jax.lax.rsqrt(v + 1e-05)


def _fold(cols, op):
    r = cols[0]
    for c in cols[1:]:
        r = op(r, c)
    r = op(r, pltpu.roll(r, 64, 1))
    return op(r, pltpu.roll(r, 32, 1))


def _phi(p):
    cols = [p[:, j * 128:(j + 1) * 128] for j in range(5)]
    mx = _fold(cols, jnp.maximum)
    mn = _fold(cols, jnp.minimum)
    ep = [jnp.exp(c - mx) for c in cols]
    en = [jnp.exp(mn - c) for c in cols]
    rp = 1.0 / _fold(ep, jnp.add)
    rn = 1.0 / _fold(en, jnp.add)
    return [e * rp for e in ep] + [e * rn for e in en]


def _kernel(x_ref, wqkv_ref, wphi_ref, woa_ref, mem0_ref, wq_hbm, wk_hbm, wv_hbm, wo_hbm,
            o_ref, xs, xn, wa, wop, kvt, sq, sk, sv, wo, wq, wk, wv, sems):
    copies = [pltpu.make_async_copy(s, d, sems.at[i]) for i, (s, d) in enumerate(
        ((wq_hbm, sq), (wk_hbm, sk), (wv_hbm, sv), (wo_hbm, wo)))]
    for c in copies:
        c.start()

    r = _iota((D, D), 0)
    c = _iota((D, D), 1)
    same = (r // FA) == (c % HA)
    sel = ((_iota((D, 32), 0) % FA) == _iota((D, 32), 1)).astype(BF16)
    rr = jnp.concatenate([wphi_ref[...], jnp.zeros((32 - FA, D), BF16)], axis=0)
    bmat = jnp.where(same, _dot(sel, rr), 0.0).astype(BF16)
    perm = jnp.logical_and(same, (r % FA) == (c // HA)).astype(BF16)
    wa[:, 0:D] = _dot(wqkv_ref[:, 0:D], bmat).astype(BF16)
    wa[:, D:2 * D] = _dot(wqkv_ref[:, D:2 * D], bmat).astype(BF16)
    wa[:, 2 * D:3 * D] = _dot(wqkv_ref[:, 2 * D:3 * D], perm).astype(BF16)
    wop[...] = _dot(perm, woa_ref[...], TN).astype(BF16)
    xs[...] = x_ref[...].astype(F32)

    def layer_a():
        kvt[...] = jnp.zeros_like(kvt)

        def keys(t, z):
            rows = pl.ds(pl.multiple_of(t * TA, TA), TA)
            h = _ln(xs[rows, :]).astype(BF16)
            xn[rows, :] = h.astype(F32)
            pkv = _dot(h, wa[:, D:3 * D])
            phi = jnp.concatenate(_phi(pkv[:, 0:D]), axis=1)
            kvt[...] += _dot(pkv[:, D:2 * D].astype(BF16), phi.astype(BF16), TN)
            return z + jnp.sum(phi, axis=0, keepdims=True)

        z = jax.lax.fori_loop(0, S // TA, keys, jnp.zeros((1, 2 * D), F32))
        msk = (_iota((D, 2 * D), 0) % HA) == (_iota((D, 2 * D), 1) % HA)
        kvb = jnp.where(msk, kvt[...], 0.0).astype(BF16)
        kw = _dot(kvb, wop[...], TN).astype(BF16)

        def queries(t, carry):
            rows = pl.ds(pl.multiple_of(t * TA, TA), TA)
            pq = _dot(xn[rows, :].astype(BF16), wa[:, 0:D])
            ph = _phi(pq)
            den = _fold([p * z[:, j * 128:(j + 1) * 128] for j, p in enumerate(ph)],
                        jnp.add) + 1e-06
            rd = 1.0 / den
            phn = jnp.concatenate([p * rd for p in ph], axis=1).astype(BF16)
            x = xs[rows, :] + _dot(phn, kw)
            xs[rows, :] = x
            xn[rows, :] = _rb(_ln(x))
            return carry

        jax.lax.fori_loop(0, S // TA, queries, 0)

    def layer_b():
        row = _iota((L, 2 * L), 0)
        col = _iota((L, 2 * L), 1)
        first = col < L
        keyi = jnp.where(first, col, col - L)
        vis = jnp.logical_or(row < M, row >= keyi)
        lane_a = _iota((L, PW), 1) < EB
        scale = EB ** (-0.5)

        def proj(h, p):
            sl = slice(p * PW, (p + 1) * PW)
            return _dot(h, wq[:, sl]), _dot(h, wk[:, sl]), _dot(h, wv[:, sl])

        def bd(a):
            return jnp.concatenate([jnp.where(lane_a, a, 0.0), jnp.where(lane_a, 0.0, a)],
                                   axis=0).astype(BF16)

        def scores(q, k):
            s = _dot(_rb(q), bd(k), NT) * scale
            s = jnp.where(vis, s, -1000000000.0)
            ma = jnp.max(jnp.where(first, s, -jnp.inf), axis=-1, keepdims=True)
            mb = jnp.max(jnp.where(first, -jnp.inf, s), axis=-1, keepdims=True)
            e = jnp.exp(s - jnp.where(first, ma, mb))
            la = jnp.sum(jnp.where(first, e, 0.0), axis=-1, keepdims=True)
            lb = jnp.sum(jnp.where(first, 0.0, e), axis=-1, keepdims=True)
            return _rb(e / jnp.where(first, la, lb))

        def step(s, mem):
            rows = pl.ds(pl.multiple_of(s * SEG, SEG), SEG)
            h = jnp.concatenate([mem, xn[rows, :]], axis=0)
            qkv, pp, oo = {}, {}, {}
            acc = None
            LAG = 3
            for i in range(NP + 2 + LAG):
                if i < NP:
                    qkv[i] = proj(h, i)
                if 0 <= i - 1 < NP:
                    pp[i - 1] = scores(qkv[i - 1][0], qkv[i - 1][1])
                if 0 <= i - 2 < NP:
                    oo[i - 2] = _rb(_dot(pp.pop(i - 2), bd(qkv.pop(i - 2)[2])))
                j = i - 2 - LAG
                if 0 <= j < NP:
                    d = _dot(oo.pop(j), wo[j * PW:(j + 1) * PW, :])
                    acc = d if acc is None else acc + d
            xs[rows, :] = xs[rows, :] + acc[M:, :]
            return _rb(acc[:M, :])

        jax.lax.fori_loop(0, S // SEG, step, mem0_ref[...].astype(F32))

    def block(it, carry):
        layer_a()

        @pl.when(it == 0)
        def _():
            for cp in copies:
                cp.wait()

            def tpose(p, carry):
                sl = pl.ds(pl.multiple_of(p * PW, 128), PW)
                for src, dst in ((sq, wq), (sk, wk), (sv, wv)):
                    dst[:, sl] = src[sl, :].T
                return carry

            jax.lax.fori_loop(0, NP, tpose, 0)

        layer_b()
        return carry

    jax.lax.fori_loop(0, 2, block, 0)
    o_ref[...] = xs[...].astype(o_ref.dtype)


@functools.partial(jax.jit, static_argnames=("B_seg_len",))
def pallas_interleave_layers__linear_kernel_hedgehog__memory_aug_recurrent_mem_tr__prompt_kernel(
    A_x, A_wqkv, A_w_phi, A_wo, B_x, B_mem0, B_Wq, B_Wk, B_Wv, B_Wo, B_seg_len,
):
    del B_x
    assert B_seg_len == SEG
    tr = lambda w: jnp.transpose(w, (1, 2, 0)).reshape(HB * EB, D)
    vm = pl.BlockSpec(memory_space=pltpu.VMEM)
    hbm = pl.BlockSpec(memory_space=pl.ANY)
    wshape = pltpu.VMEM((HB * EB, D), BF16)
    wt = pltpu.VMEM((D, HB * EB), BF16)
    out = pl.pallas_call(
        _kernel,
        out_shape=jax.ShapeDtypeStruct((S, D), A_x.dtype),
        in_specs=[vm] * 5 + [hbm] * 4,
        out_specs=vm,
        scratch_shapes=[
            pltpu.VMEM((S, D), F32), pltpu.VMEM((S, D), F32),
            pltpu.VMEM((D, 3 * D), BF16), pltpu.VMEM((D, D), BF16),
            pltpu.VMEM((D, 2 * D), F32),
            wshape, wshape, wshape, wshape, wt, wt, wt,
            pltpu.SemaphoreType.DMA((4,)),
        ],
        compiler_params=pltpu.CompilerParams(vmem_limit_bytes=110 * 1024 * 1024),
    )(
        A_x.reshape(S, D), A_wqkv,
        jnp.transpose(A_w_phi, (1, 2, 0)).reshape(FA, FA * HA), A_wo,
        B_mem0.reshape(M, D), tr(B_Wq), tr(B_Wk), tr(B_Wv), B_Wo.reshape(HB * EB, D),
    )
    return out.reshape(A_x.shape)
```

```python
import functools

import jax
import jax.numpy as jnp
import jax.experimental.pallas as pl
import jax.experimental.pallas.tpu as pltpu

F32 = jnp.float32
BF16 = jnp.bfloat16
U32 = jnp.uint32

S, D = 2048, 640
HA, FA = 32, 20
HB, EB = 32, 192
M, SEG = 8, 32
L = M + SEG
TA = 256
PW = 2 * EB
NP = HB // 2
G, L1, L2, L3 = 4, 0, 1, 1

NT = (((1,), (1,)), ((), ()))
NN = (((1,), (0,)), ((), ()))
TN = (((0,), (0,)), ((), ()))


def _dot(a, b, dims=NN):
    return jax.lax.dot_general(a, b, dims, preferred_element_type=F32)


def _iota(shape, axis):
    return jax.lax.broadcasted_iota(jnp.int32, shape, axis)


def _rb(x):
    return x.astype(BF16).astype(F32)


def _w(x):
    return pltpu.bitcast(x, BF16)


def _ln(x):
    m = jnp.mean(x, axis=-1, keepdims=True)
    c = x - m
    v = jnp.mean(c * c, axis=-1, keepdims=True)
    return c * jax.lax.rsqrt(v + 1e-05)


def _fold(cols, op):
    r = cols[0]
    for c in cols[1:]:
        r = op(r, c)
    r = op(r, pltpu.roll(r, 64, 1))
    return op(r, pltpu.roll(r, 32, 1))


def _phi(p):
    cols = [p[:, j * 128:(j + 1) * 128] for j in range(5)]
    mx = _fold(cols, jnp.maximum)
    mn = _fold(cols, jnp.minimum)
    ep = [jnp.exp(c - mx) for c in cols]
    en = [jnp.exp(mn - c) for c in cols]
    rp = 1.0 / _fold(ep, jnp.add)
    rn = 1.0 / _fold(en, jnp.add)
    return [e * rp for e in ep] + [e * rn for e in en]


def _kernel(x_ref, wqkv_ref, wphi_ref, woa_ref, mem0_ref, wq_hbm, wk_hbm, wv_hbm, wo_hbm,
            o_ref, xs, xn, wa, wop, kvt, sq, sk, sv, so, wo, wq, wk, wv, sems):
    copies = [pltpu.make_async_copy(s, d, sems.at[i]) for i, (s, d) in enumerate(
        ((wq_hbm, sq), (wk_hbm, sk), (wv_hbm, sv), (wo_hbm, so)))]
    for c in copies:
        c.start()

    r = _iota((D, D), 0)
    c = _iota((D, D), 1)
    same = (r // FA) == (c % HA)
    sel = ((_iota((D, 32), 0) % FA) == _iota((D, 32), 1)).astype(BF16)
    rr = jnp.concatenate([wphi_ref[...], jnp.zeros((32 - FA, D), BF16)], axis=0)
    bmat = jnp.where(same, _dot(sel, rr), 0.0).astype(BF16)
    perm = jnp.logical_and(same, (r % FA) == (c // HA)).astype(BF16)
    wa[:, 0:D] = pltpu.bitcast(_dot(wqkv_ref[:, 0:D], bmat).astype(BF16), U32)
    wa[:, D:2 * D] = pltpu.bitcast(_dot(wqkv_ref[:, D:2 * D], bmat).astype(BF16), U32)
    wa[:, 2 * D:3 * D] = pltpu.bitcast(_dot(wqkv_ref[:, 2 * D:3 * D], perm).astype(BF16), U32)
    wop[...] = _dot(perm, woa_ref[...], TN).astype(BF16)
    xs[...] = x_ref[...].astype(F32)

    def layer_a():
        kvt[...] = jnp.zeros_like(kvt)

        def keys(t, z):
            rows = pl.ds(pl.multiple_of(t * TA, TA), TA)
            h = _ln(xs[rows, :]).astype(BF16)
            xn[rows, :] = h.astype(F32)
            pkv = _dot(h, _w(wa[:, D:3 * D]))
            phi = jnp.concatenate(_phi(pkv[:, 0:D]), axis=1)
            kvt[...] += _dot(pkv[:, D:2 * D].astype(BF16), phi.astype(BF16), TN)
            return z + jnp.sum(phi, axis=0, keepdims=True)

        z = jax.lax.fori_loop(0, S // TA, keys, jnp.zeros((1, 2 * D), F32), unroll=2)
        msk = (_iota((D, 2 * D), 0) % HA) == (_iota((D, 2 * D), 1) % HA)
        kvb = jnp.where(msk, kvt[...], 0.0).astype(BF16)
        kw = _dot(kvb, wop[...], TN).astype(BF16)

        def queries(t, carry):
            rows = pl.ds(pl.multiple_of(t * TA, TA), TA)
            pq = _dot(xn[rows, :].astype(BF16), _w(wa[:, 0:D]))
            ph = _phi(pq)
            den = _fold([p * z[:, j * 128:(j + 1) * 128] for j, p in enumerate(ph)],
                        jnp.add) + 1e-06
            rd = 1.0 / den
            phn = jnp.concatenate([p * rd for p in ph], axis=1).astype(BF16)
            x = xs[rows, :] + _dot(phn, kw)
            xs[rows, :] = x
            xn[rows, :] = _rb(_ln(x))
            return carry

        jax.lax.fori_loop(0, S // TA, queries, 0, unroll=2)

    def layer_b():
        row = _iota((L, 2 * L), 0)
        col = _iota((L, 2 * L), 1)
        first = col < L
        keyi = jnp.where(first, col, col - L)
        vis = jnp.logical_or(row < M, row >= keyi)
        lane_a = _iota((L, PW), 1) < EB
        scale = EB ** (-0.5)

        def bd(a):
            return jnp.concatenate([jnp.where(lane_a, a, 0.0), jnp.where(lane_a, 0.0, a)],
                                   axis=0).astype(BF16)

        def scores(q, k):
            s = _dot(_rb(q), bd(k), NT) * scale
            s = jnp.where(vis, s, -1000000000.0)
            ma = jnp.max(jnp.where(first, s, -jnp.inf), axis=-1, keepdims=True)
            mb = jnp.max(jnp.where(first, -jnp.inf, s), axis=-1, keepdims=True)
            e = jnp.exp(s - jnp.where(first, ma, mb))
            la = jnp.sum(jnp.where(first, e, 0.0), axis=-1, keepdims=True)
            lb = jnp.sum(jnp.where(first, 0.0, e), axis=-1, keepdims=True)
            return _rb(e / jnp.where(first, la, lb))

        def step(s, mem):
            rows = pl.ds(pl.multiple_of(s * SEG, SEG), SEG)
            h = jnp.concatenate([mem, xn[rows, :]], axis=0)
            qkv, pp, oo = {}, {}, {}
            acc = None
            ng, gw = NP // G, G * PW
            sub = lambda a, u: a[:, u * PW:(u + 1) * PW]
            for i in range(ng + L3):
                if i < ng:
                    qkv[i] = [_dot(h, _w(w[:, i * gw:(i + 1) * gw])) for w in (wk, wq, wv)]
                if 0 <= i - L1 < ng:
                    k, q, _ = qkv[i - L1]
                    pp[i - L1] = [scores(sub(q, u), sub(k, u)) for u in range(G)]
                if 0 <= i - L2 < ng:
                    v = qkv.pop(i - L2)[2]
                    oo[i - L2] = _rb(jnp.concatenate(
                        [_dot(p, bd(sub(v, u))) for u, p in enumerate(pp.pop(i - L2))], axis=1))
                j = i - L3
                if 0 <= j < ng:
                    d = _dot(oo.pop(j), _w(wo[j * gw // 2:(j + 1) * gw // 2, :]))
                    acc = d if acc is None else acc + d
            xs[rows, :] = xs[rows, :] + acc[M:, :]
            return _rb(acc[:M, :])

        jax.lax.fori_loop(0, S // SEG, step, mem0_ref[...].astype(F32))

    def block(it, carry):
        layer_a()

        @pl.when(it == 0)
        def _():
            for cp in copies:
                cp.wait()

            def tpose(p, carry):
                sl = pl.ds(pl.multiple_of(p * PW, 128), PW)
                for src, dst in ((sq, wq), (sk, wk), (sv, wv)):
                    dst[:, sl] = pltpu.bitcast(src[sl, :].T, U32)
                wo[pl.ds(pl.multiple_of(p * EB, 8), EB), :] = pltpu.bitcast(so[sl, :], U32)
                return carry

            jax.lax.fori_loop(0, NP, tpose, 0)

        layer_b()
        return carry

    jax.lax.fori_loop(0, 2, block, 0)
    o_ref[...] = xs[...].astype(o_ref.dtype)


@functools.partial(jax.jit, static_argnames=("B_seg_len",))
def pallas_interleave_layers__linear_kernel_hedgehog__memory_aug_recurrent_mem_tr__prompt_kernel(
    A_x, A_wqkv, A_w_phi, A_wo, B_x, B_mem0, B_Wq, B_Wk, B_Wv, B_Wo, B_seg_len,
):
    del B_x
    assert B_seg_len == SEG
    tr = lambda w: jnp.transpose(w, (1, 2, 0)).reshape(HB * EB, D)
    vm = pl.BlockSpec(memory_space=pltpu.VMEM)
    hbm = pl.BlockSpec(memory_space=pl.ANY)
    wshape = pltpu.VMEM((HB * EB, D), BF16)
    wt = pltpu.VMEM((D // 2, HB * EB), U32)
    out = pl.pallas_call(
        _kernel,
        out_shape=jax.ShapeDtypeStruct((S, D), A_x.dtype),
        in_specs=[vm] * 5 + [hbm] * 4,
        out_specs=vm,
        scratch_shapes=[
            pltpu.VMEM((S, D), F32), pltpu.VMEM((S, D), F32),
            pltpu.VMEM((D // 2, 3 * D), U32), pltpu.VMEM((D, D), BF16),
            pltpu.VMEM((D, 2 * D), F32),
            wshape, wshape, wshape, wshape, pltpu.VMEM((HB * EB // 2, D), U32), wt, wt, wt,
            pltpu.SemaphoreType.DMA((4,)),
        ],
        compiler_params=pltpu.CompilerParams(vmem_limit_bytes=110 * 1024 * 1024),
    )(
        A_x.reshape(S, D), A_wqkv,
        jnp.transpose(A_w_phi, (1, 2, 0)).reshape(FA, FA * HA), A_wo,
        B_mem0.reshape(M, D), tr(B_Wq), tr(B_Wk), tr(B_Wv), B_Wo.reshape(HB * EB, D),
    )
    return out.reshape(A_x.shape)
```
